```python
import os as _os
_os.environ.setdefault("JAX_PLATFORMS", "cpu")
import jax
import jax.numpy as jnp

def _softmax(x, axis=-1):
    return jax.nn.softmax(x, axis=axis)
def _gelu(x):
    return jax.nn.gelu(x, approximate=True)
def _silu(x):
    return jax.nn.silu(x)
def _sigmoid(x):
    return jax.nn.sigmoid(x)
def _layernorm(x, axis=-1, eps=1e-5):
    m = jnp.mean(x, axis=axis, keepdims=True)
    v = jnp.var(x, axis=axis, keepdims=True)
    return (x - m) / jnp.sqrt(v + eps)
def _scatter_add(tgt, idx, src, axis=0):
    return tgt.at[idx].add(src)
def _segment_sum(src, seg, n):
    return jax.ops.segment_sum(src, seg, n)
class _Rng:
    def __init__(self, key):
        self._k = key
    def _next(self):
        self._k, sub = jax.random.split(self._k)
        return sub
    def normal(self, shape):
        return jax.random.normal(self._next(), shape, dtype=jnp.bfloat16)
    def randint(self, lo, hi, shape):
        return jax.random.randint(self._next(), shape, lo, hi, dtype=jnp.int32)
    def uniform(self, shape, lo=0.0, hi=1.0):
        return jax.random.uniform(self._next(), shape, jnp.bfloat16, lo, hi)
    def permutation(self, n):
        return jax.random.permutation(self._next(), n)


kernel_name = 'gated_mix__compressed_kv_cla__ssm_conv_h3__prompt'

def setup_inputs():
    _rng = _Rng(jax.random.key(int.from_bytes(__import__("os").urandom(4), "little")))
    _w = (lambda a: (lambda t: t.astype(jnp.bfloat16) if jnp.issubdtype(t.dtype, jnp.floating) else t)(jnp.asarray(a)))
    def _A_setup():
        B, H, Sq, Sk, D, M = 1, 32, 2048, 2048, 128, 1024
        Dc = 4 * D
        return {
            "x": _w((lambda *s: _rng.normal(s) * 0.05)(B, Sq, M)),
            "c_kv": _w((lambda *s: _rng.normal(s) * 0.8)(B, Sk, Dc)),
            "w_q": _w((lambda *s: _rng.normal(s) * 3.2)(M, H, D) * (M ** -0.5)),
            "w_uk": _w((lambda *s: _rng.normal(s) * 3.2)(Dc, H, D) * (Dc ** -0.5)),
            "w_uv": _w((lambda *s: _rng.normal(s) * 0.8)(Dc, H, D) * (Dc ** -0.5)),
            "w_o": _w((lambda *s: _rng.normal(s) * 0.8)(H, D, M) * ((H * D) ** -0.5)),
        }
    _A_in = _A_setup()

    def _B_setup():
        B, S, D = 1, 2048, 1024
        ks = 4
        return {
            "q": _w((lambda *s: _rng.normal(s) * 0.05)(B, S, D)),
            "k": _w((lambda *s: _rng.normal(s) * 0.8)(B, S, D)),
            "v": _w((lambda *s: _rng.normal(s) * 0.8)(B, S, D)),
            "shift_k": _w((lambda *s: _rng.normal(s) * 0.8)(D, ks) * 0.5),
            "ssm_k": _w((lambda *s: _rng.normal(s) * 0.8)(D, S) * (1.0 / S ** 0.5)),
            "ssm_D": _w((lambda *s: _rng.normal(s) * 0.8)(D)),
        }
    _B_in = _B_setup()

    return {
        "A_x": _A_in["x"],
        "A_c_kv": _A_in["c_kv"],
        "A_w_q": _A_in["w_q"],
        "A_w_uk": _A_in["w_uk"],
        "A_w_uv": _A_in["w_uv"],
        "A_w_o": _A_in["w_o"],
        "B_q": _B_in["q"],
        "B_k": _B_in["k"],
        "B_v": _B_in["v"],
        "B_shift_k": _B_in["shift_k"],
        "B_ssm_k": _B_in["ssm_k"],
        "B_ssm_D": _B_in["ssm_D"],
        "gate_w": _w((lambda *s: _rng.normal(s) * 0.05)(1024) * 16.0),
    }

def reference(A_x, A_c_kv, A_w_q, A_w_uk, A_w_uv, A_w_o, B_q, B_k, B_v, B_shift_k, B_ssm_k, B_ssm_D, gate_w):
    def _A_ref(x, c_kv, w_q, w_uk, w_uv, w_o):
        B, Sq, M = x.shape[0], x.shape[1], x.shape[2]
        Sk = c_kv.shape[1]
        H, D = w_q.shape[1], w_q.shape[2]
        q = jnp.einsum("bqm,mhd->bhqd", x, w_q)
        k = jnp.einsum("bkc,chd->bhkd", c_kv, w_uk)
        v = jnp.einsum("bkc,chd->bhkd", c_kv, w_uv)
        scores = jnp.einsum("bhqd,bhkd->bhqk", q, k) * (D ** -0.5)
        off = Sk - Sq
        qi = jnp.arange(Sq)[:, None]
        kj = jnp.arange(Sk)[None, :]
        cmask = kj <= (qi + off)
        scores = jnp.where(cmask[None, None], scores, -1e9)
        p = _softmax(scores, axis=-1)
        ctx = jnp.einsum("bhqk,bhkd->bhqd", p, v)
        return jnp.einsum("bhqd,hdm->bqm", ctx, w_o)

    def _B_ref(q, k, v, shift_k, ssm_k, ssm_D):
        B, S, D = q.shape
        ks = shift_k.shape[-1]
        k_pad = jnp.pad(k, ((0, 0), (ks - 1, 0), (0, 0)))
        k_shift = jnp.zeros_like(k)
        for t in range(ks):
            k_shift = k_shift + k_pad[:, t:t + S, :] * shift_k[:, ks - 1 - t][None, None, :]
        kv = k_shift * v
        L = 2 * S
        kv_pad = jnp.pad(kv, ((0, 0), (0, S), (0, 0)))
        kf_pad = jnp.pad(ssm_k, ((0, 0), (0, S)))
        kv_f = (lambda x, axes=(-2,-1): jnp.fft.rfft2(x.astype(jnp.float32), axes=axes))(kv_pad[:, None, :, :], axes=(1, 2))
        kf_f = (lambda x, axes=(-2,-1): jnp.fft.rfft2(x.astype(jnp.float32), axes=axes))(kf_pad[:, None, :], axes=(1, 2))
        kf_f = (lambda x, *d: x.transpose(*d))(kf_f, 1, 2, 0)
        y_f = kv_f * kf_f[None, :, :, :]
        y = (lambda x, s, axes=(-2,-1): jnp.fft.irfft2(x, s=s, axes=axes).astype(jnp.bfloat16))(y_f, (1, L), axes=(1, 2))[:, 0, :S, :]
        y = y + kv * ssm_D[None, None, :]
        return q * y

    x = A_x
    g = _sigmoid((x * gate_w).sum(-1, keepdims=True))
    a = _A_ref(x, A_c_kv, A_w_q, A_w_uk, A_w_uv, A_w_o)
    b = _B_ref(x, B_k, B_v, B_shift_k, B_ssm_k, B_ssm_D)
    return g * a + (1 - g) * b
```

```python
import functools
import numpy as np
import jax
import jax.numpy as jnp
from jax import lax
import jax.experimental.pallas as pl
import jax.experimental.pallas.tpu as pltpu

S = 2048
M = 1024
H = 32
DH = 128
DC = 512
T = 128
NT = S // T
NCB = M // T
C = 128
NCH = S // C

BF = jnp.bfloat16
F32 = jnp.float32


def _dft_matrix():
    n = 2 * C
    f = np.concatenate([np.arange(0, C, 2), np.arange(1, C, 2)])
    r = np.arange(C)
    ang = np.pi * (((2 * f[:, None] + 1) * r[None, :]) % (2 * n)) / n
    return np.concatenate([np.cos(ang), -np.sin(ang)], axis=0).astype(np.float32)

_F = _dft_matrix()
_G = np.ascontiguousarray(_F.T) * np.float32(1.0 / C)

NT_DIMS = (((1,), (1,)), ((), ()))

def _dot(a, b):
    return jnp.dot(a, b, preferred_element_type=F32)

def _dot_nt(a, b):
    return lax.dot_general(a, b, NT_DIMS, preferred_element_type=F32)

def _head_w(w_ref, rows, h):
    w32 = w_ref.bitcast(jnp.uint32)
    u = w32[pl.ds(lax.shift_right_logical(h, 1), rows, stride=H // 2), :]
    sh = (16 - 16 * (h & 1)).astype(jnp.uint32)
    u = (u << sh) & jnp.uint32(0xFFFF0000)
    return pltpu.bitcast(u, F32).astype(BF)


def make(G=2, order="fwd"):
    BQ = G * T
    NB = S // BQ

    def attn_head(h, x_ref, c_ref, wq_ref, wuk_ref, wuv_ref, ctx_ref):
        hg = h & 7
        wq = wq_ref[hg]
        wuk = wuk_ref[hg]
        wuv = wuv_ref[hg]
        scale = np.float32(DH ** -0.5 * np.log2(np.e))
        row = lax.broadcasted_iota(jnp.int32, (T, T), 0)
        col = lax.broadcasted_iota(jnp.int32, (T, T), 1)
        causal = col <= row
        q = {}; k = {}; v = {}; s = {}; p = {}; linv = {}

        def proj_q(i):
            q[i] = (_dot(x_ref[i * BQ:(i + 1) * BQ, :], wq) * scale).astype(BF)
        def proj_k(i):
            kk = _dot(c_ref[i * BQ:(i + 1) * BQ, :], wuk).astype(BF)
            for a in range(G):
                k[i * G + a] = kk[a * T:(a + 1) * T]
        def proj_v(i):
            vv = _dot(c_ref[i * BQ:(i + 1) * BQ, :], wuv).astype(BF)
            for a in range(G):
                v[i * G + a] = vv[a * T:(a + 1) * T]
        def qk(i):
            for j in range((i + 1) * G):
                a0 = max(0, j - i * G)
                r = _dot_nt(q[i][a0 * T:], k[j])
                for a in range(a0, G):
                    t = i * G + a
                    blk = r[(a - a0) * T:(a - a0 + 1) * T]
                    if t == j:
                        blk = jnp.where(causal, blk, -1e30)
                    s[t, j] = blk
        def softmax(i):
            ms = []
            for a in range(G):
                t = i * G + a
                m = s[t, 0]
                for j in range(1, t + 1):
                    m = jnp.maximum(m, s[t, j])
                ms.append(jnp.max(m, axis=1, keepdims=True))
            ls = [None] * G
            for j in range((i + 1) * G):
                for a in range(max(0, j - i * G), G):
                    t = i * G + a
                    e = jnp.exp2(s[t, j] - ms[a])
                    ls[a] = e if ls[a] is None else ls[a] + e
                    p[t, j] = e.astype(BF)
            for a in range(G):
                linv[i * G + a] = 1.0 / jnp.sum(ls[a], axis=1, keepdims=True)
        def pv(i):
            o = [None] * G
            for j in range((i + 1) * G):
                a0 = max(0, j - i * G)
                pp = jnp.concatenate([p[i * G + a, j] for a in range(a0, G)], axis=0)
                r = _dot(pp, v[j])
                for a in range(a0, G):
                    blk = r[(a - a0) * T:(a - a0 + 1) * T]
                    o[a] = blk if o[a] is None else o[a] + blk
            for a in range(G):
                t = i * G + a
                ctx_ref[h, t * T:(t + 1) * T, :] = (o[a] * linv[t]).astype(BF)

        if order == "fwd":
            proj_k(0); proj_q(0); proj_k(1); qk(0); proj_q(1)
            for i in range(NB):
                proj_v(i)
                if i + 2 < NB:
                    proj_k(i + 2)
                if i + 1 < NB:
                    qk(i + 1)
                softmax(i)
                if i + 2 < NB:
                    proj_q(i + 2)
                pv(i)
        else:
            for i in range(NB):
                proj_k(i)
            proj_q(NB - 1)
            proj_q(NB - 2)
            qk(NB - 1)
            for i in range(NB):
                proj_v(i)
            for i in reversed(range(NB)):
                if i >= 1:
                    qk(i - 1)
                softmax(i)
                if i >= 2:
                    proj_q(i - 2)
                pv(i)

    def out_block(cb, x_ref, xc_ref, wo_ref, bk_ref, bv_ref, sk_ref, sh_ref, d_ref, f_ref, gm_ref,
                  o_ref, ctx_ref, g_ref, kp_ref, u_ref, kf_ref, z_ref, kv_ref):
        kp_ref[0:8, :] = jnp.zeros((8, T), F32)
        kp_ref[8:8 + S, :] = bk_ref[...].astype(F32)
        shw = sh_ref[...].astype(F32)
        fm = f_ref[...]
        for j in range(NCH):
            ks = None
            for t in range(4):
                term = kp_ref[8 + j * C - t:8 + (j + 1) * C - t, :] * shw[t:t + 1, :]
                ks = term if ks is None else ks + term
            kv = (ks * bv_ref[j * C:(j + 1) * C, :].astype(F32)).astype(BF)
            kv_ref[j * C:(j + 1) * C, :] = kv
            u_ref[j] = _dot(fm, kv)
        prev = None
        hc = C // 2
        for m in range(NCH):
            cur = _dot_nt(fm, sk_ref[:, m * C:(m + 1) * C])
            if prev is None:
                kf_ref[m] = cur
            else:
                kf_ref[m, 0:hc] = cur[0:hc] - prev[C:C + hc]
                kf_ref[m, hc:C] = cur[hc:C] + prev[C + hc:2 * C]
                kf_ref[m, C:C + hc] = cur[C:C + hc] + prev[0:hc]
                kf_ref[m, C + hc:] = cur[C + hc:] - prev[hc:C]
            prev = cur
        RB = 16
        def mac(fb):
            r0 = fb * RB
            for i in range(NCH):
                zr = zi = None
                for j in range(i + 1):
                    ur = u_ref[j, r0:r0 + RB]; ui = u_ref[j, C + r0:C + r0 + RB]
                    kr = kf_ref[i - j, r0:r0 + RB]; ki = kf_ref[i - j, C + r0:C + r0 + RB]
                    tr = ur * kr - ui * ki
                    ti = ur * ki + ui * kr
                    zr = tr if zr is None else zr + tr
                    zi = ti if zi is None else zi + ti
                z_ref[i, r0:r0 + RB] = zr.astype(BF)
                z_ref[i, C + r0:C + r0 + RB] = zi.astype(BF)
        RO = 512
        a_out = []
        nfb = C // RB
        for rb in range(S // RO):
            for fb in range(rb * nfb // (S // RO), (rb + 1) * nfb // (S // RO)):
                mac(fb)
            acc = None
            for hh in range(H):
                r = _dot(ctx_ref[hh, rb * RO:(rb + 1) * RO, :], wo_ref[hh * DH:(hh + 1) * DH, :])
                acc = r if acc is None else acc + r
            a_out.append(acc)
        gm = gm_ref[...]
        dd = d_ref[pl.ds(cb, 1), :]
        for i in range(NCH):
            y = _dot(gm, z_ref[i])
            rows = slice(i * C, (i + 1) * C)
            y = y + kv_ref[rows, :].astype(F32) * dd
            b = xc_ref[rows, :].astype(F32) * y
            a = a_out[i * C // RO][(i * C) % RO:(i * C) % RO + C]
            g = g_ref[rows, :]
            o_ref[rows, :] = (g * a + (1.0 - g) * b).astype(BF)

    def kernel(x_ref, c_ref, wq_ref, wuk_ref, wuv_ref, wo_ref, xc_ref, bk_ref, bv_ref, sk_ref, sh_ref,
               d_ref, gw_ref, f_ref, gm_ref, o_ref,
               ctx_ref, g_ref, kp_ref, u_ref, kf_ref, z_ref, kv_ref, d32_ref, wq_s, wuk_s, wuv_s):
        step = pl.program_id(0)

        @pl.when(step == 0)
        def _():
            gw = gw_ref[...].astype(F32)
            d32_ref[...] = d_ref[...].astype(F32)
            for rb in range(S // 256):
                acc = None
                for cb in range(NCB):
                    t = x_ref[rb * 256:(rb + 1) * 256, cb * T:(cb + 1) * T].astype(F32) * gw[cb:cb + 1, :]
                    acc = t if acc is None else acc + t
                z = jnp.sum(acc, axis=1, keepdims=True)
                g_ref[rb * 256:(rb + 1) * 256, :] = jnp.broadcast_to(jax.nn.sigmoid(z), (256, T))

        @pl.when((step & 39) == 0)
        def _():
            for src, dst, rows in ((wq_ref, wq_s, M), (wuk_ref, wuk_s, DC), (wuv_ref, wuv_s, DC)):
                for r0 in range(0, rows, 256):
                    w = src[r0:r0 + 256].reshape(256, 8 * DH)
                    for hh in range(8):
                        dst[hh, r0:r0 + 256, :] = w[:, hh * DH:(hh + 1) * DH]

        @pl.when(step < H)
        def _():
            attn_head(step, x_ref, c_ref, wq_s, wuk_s, wuv_s, ctx_ref)

        @pl.when(step >= H)
        def _():
            out_block(step - H, x_ref, xc_ref, wo_ref, bk_ref, bv_ref, sk_ref, sh_ref, d32_ref, f_ref, gm_ref,
                      o_ref, ctx_ref, g_ref, kp_ref, u_ref, kf_ref, z_ref, kv_ref)

    @jax.jit
    def run(A_x, A_c_kv, A_w_q, A_w_uk, A_w_uv, A_w_o, B_q, B_k, B_v, B_shift_k, B_ssm_k, B_ssm_D, gate_w):
        del B_q
        x = A_x.reshape(S, M)
        def full(shape):
            return pl.BlockSpec(shape, lambda i: (0,) * len(shape), pipeline_mode=pl.Buffered(1))
        cbi = lambda i: jnp.maximum(i - H, 0)
        col = lambda rows: pl.BlockSpec((rows, T), lambda i: (0, cbi(i)))
        wsp = lambda rows: pl.BlockSpec((rows, 8, DH), lambda i: (0, jnp.minimum(i // 8, 3), 0))
        out = pl.pallas_call(
            kernel,
            grid=(H + NCB,),
            in_specs=[full((S, M)), full((S, DC)), wsp(M), wsp(DC), wsp(DC),
                      col(H * DH), col(S), col(S), col(S),
                      pl.BlockSpec((T, S), lambda i: (cbi(i), 0)), col(4),
                      full((NCB, T)), full((NCB, T)), full((2 * C, C)), full((C, 2 * C))],
            out_specs=col(S),
            out_shape=jax.ShapeDtypeStruct((S, M), BF),
            scratch_shapes=[pltpu.VMEM((H, S, DH), BF), pltpu.VMEM((S, T), F32), pltpu.VMEM((S + 8, T), F32),
                            pltpu.VMEM((NCH, 2 * C, T), F32), pltpu.VMEM((NCH, 2 * C, T), F32),
                            pltpu.VMEM((NCH, 2 * C, T), BF), pltpu.VMEM((S, T), BF), pltpu.VMEM((NCB, T), F32),
                            pltpu.VMEM((8, M, DH), BF), pltpu.VMEM((8, DC, DH), BF), pltpu.VMEM((8, DC, DH), BF)],
            compiler_params=pltpu.CompilerParams(dimension_semantics=("arbitrary",), vmem_limit_bytes=120 * 2 ** 20),
            name="gmix",
        )(x, A_c_kv.reshape(S, DC), A_w_q, A_w_uk, A_w_uv,
          A_w_o.reshape(H * DH, M), x, B_k.reshape(S, M), B_v.reshape(S, M), B_ssm_k, B_shift_k.T,
          B_ssm_D.reshape(NCB, T), gate_w.reshape(NCB, T), jnp.asarray(_F, BF), jnp.asarray(_G, BF))
        return out.reshape(1, S, M)
    return run


pallas_gated_mix__compressed_kv_cla__ssm_conv_h3__prompt_kernel = make()
```

```python
import numpy as np
import jax
import jax.numpy as jnp
from jax import lax
import jax.experimental.pallas as pl
import jax.experimental.pallas.tpu as pltpu

S = 2048
M = 1024
H = 32
DH = 128
DC = 512
KS = 4
T = 128
NT = S // T
NB = NT // 2
NCB = M // T
HG = 8
NG = H // HG
C = 512
NCH = S // C
PH = C // 8
RO = 512

BF = jnp.bfloat16
F32 = jnp.float32
U32 = jnp.uint32
HI16 = np.uint32(0xFFFF0000)


def _dft_matrices():
    n = 2 * C
    even = np.arange(0, T, 2)
    base = np.concatenate([even, T - 1 - even])

    def mat(f, t):
        ang = np.pi * (((2 * f[:, None] + 1) * t[None, :]) % (2 * n)) / n
        re = np.cos(ang).reshape(-1, 1, 8, len(t))
        im = -np.sin(ang).reshape(-1, 1, 8, len(t))
        return np.concatenate([re, im], axis=1).reshape(-1, len(t))

    t0 = 8 * np.arange(PH)
    fwd = np.stack([mat(base, np.concatenate([t0 + r, t0 + r + 4])) for r in range(4)])
    inv = np.stack([mat(even, t0 + r).T / C for r in range(8)])
    return fwd.astype(np.float32).astype(BF), inv.astype(np.float32).astype(BF)


_FWD, _INV = _dft_matrices()


def _dot(a, b):
    return jnp.dot(a, b, preferred_element_type=F32)


def _dot_nt(a, b):
    return lax.dot_general(a, b, (((1,), (1,)), ((), ())), preferred_element_type=F32)


def _sum(xs):
    acc = xs[0]
    for v in xs[1:]:
        acc = acc + v
    return acc


def _cat(xs):
    return jnp.concatenate(list(xs), axis=0)


def _weave(a, b):
    return [v for pair in zip(a, b) for v in pair] + a[len(b):] + b[len(a):]


_LHS = ((0, 1, 3), (2, 1, 3), (0,), (3,), (0, 1, 1), (2, -1, 0), (1, -1, 3))
_RHS = ((0, 1, 3), (0,), (1, -1, 3), (2, -1, 0), (3,), (0, 1, 1), (2, 1, 3))
_SUMS = (0, 1, 4, 5, 6)
_ORDER = (1, 3, 0, 6, 4, 2, 5)


def _operand(spec, block):
    if len(spec) == 1:
        return block(spec[0])
    a, b = block(spec[0]).astype(F32), block(spec[2]).astype(F32)
    return a + b if spec[1] > 0 else a - b


def _strassen(prod):
    m2 = prod(1)
    m4 = prod(3)
    c21 = m2 + m4
    m1 = prod(0)
    a = m1 - m2
    b = m1 + m4 + prod(6)
    m5 = prod(4)
    c11 = b - m5
    m3 = prod(2)
    c12 = m3 + m5
    c22 = a + m3 + prod(5)
    return c11, c12, c21, c22


def _dft4(x, sign):
    (r0, i0), (r1, i1), (r2, i2), (r3, i3) = x
    ar, ai, br, bi = r0 + r2, i0 + i2, r0 - r2, i0 - i2
    cr, ci, dr, di = r1 + r3, i1 + i3, r1 - r3, i1 - i3
    p, m = (br - di, bi + dr), (br + di, bi - dr)
    return [(ar + cr, ai + ci), p if sign > 0 else m, (ar - cr, ai - ci), m if sign > 0 else p]


def _fold(wa, wb):
    h = np.float32(np.sqrt(0.5))
    (r0, i0), (r1, i1), (r2, i2), (r3, i3) = wb
    tw = [(r0, i0), ((r1 - i1) * h, (r1 + i1) * h), None, ((r3 + i3) * -h, (r3 - i3) * h)]
    out = [None] * 8
    for r in range(4):
        ar, ai = wa[r]
        if r == 2:
            out[r], out[r + 4] = (ar - i2, ai - r2), (ar + i2, ai + r2)
        else:
            out[r], out[r + 4] = (ar + tw[r][0], ai - tw[r][1]), (ar - tw[r][0], ai + tw[r][1])
    return out


def _halves(u):
    return pltpu.bitcast(u << 16, F32), pltpu.bitcast(u & HI16, F32)


def _pacing(loop_index):
    zero = lax.shift_right_logical(loop_index, 8)

    def after(v, dep):
        if v.dtype == BF:
            return pltpu.bitcast(after(pltpu.bitcast(v, jnp.int32), pltpu.bitcast(dep, jnp.int32)), BF)
        return jnp.where(lax.broadcasted_iota(jnp.int32, v.shape, 1) >= zero, v, dep)

    return zero, after


def _kernel(x_hbm, c_hbm, wq_hbm, wuk_hbm, wuv_hbm, wo_hbm, bk_hbm, bv_hbm, sk_hbm,
            sh_hbm, d_hbm, gw_hbm, fwd_hbm, inv_hbm, o_hbm,
            fwd_s, inv_s, x_s, c_s, wq_s, wkv_s, wo_s, bk_s, bv_s, sk_s, o_s, y32,
            kv_s, ctx7, wq7, x5, c7, wkv7, w32, g_s, k32, v32, h32, z_s, uk_s, p_s,
            q0, q1, q2, q3, s0, s1, s2, sh_s, sh_in, d_s, d_in, gw_s, sems):
    def heads_of(g):
        return pl.ds(pl.multiple_of(g * HG, HG), HG)

    def chans_of(cb):
        return pl.ds(pl.multiple_of(cb * T, T), T)

    def cp_c():
        return pltpu.make_async_copy(c_hbm, c_s, sems.at[0])

    def cp_x():
        return [pltpu.make_async_copy(x_hbm.at[:, chans_of(t)], x_s.at[t], sems.at[1]) for t in range(NCB)]

    def cp_small():
        pairs = ((sh_hbm, sh_in), (d_hbm, d_in), (gw_hbm, gw_s), (fwd_hbm, fwd_s), (inv_hbm, inv_s))
        return [pltpu.make_async_copy(a, b, sems.at[2]) for a, b in pairs]

    def cp_wo(cb):
        return pltpu.make_async_copy(wo_hbm.at[:, chans_of(cb)], wo_s.at[cb], sems.at[3])

    def cp_out(cb, rb):
        rows = pl.ds(pl.multiple_of(rb * 2 * RO, 2 * RO), 2 * RO)
        return pltpu.make_async_copy(o_s.at[cb, rows], o_hbm.at[rows, chans_of(cb)], sems.at[4])

    def cp_wkv(g, e):
        return pltpu.make_async_copy((wuk_hbm, wuv_hbm)[e].at[:, heads_of(g), :], wkv_s.at[e], sems.at[5 + e])

    def cp_early(g, e):
        return [pltpu.make_async_copy(src.at[:, chans_of(2 * g + e)], dst.at[e], sems.at[7 + e])
                for src, dst in ((bk_hbm, bk_s), (bv_hbm, bv_s))]

    def cp_late(g, e):
        hq = M // 4
        sem = sems.at[9 + e]
        return [pltpu.make_async_copy(wq_hbm.at[pl.ds((k + e) * hq, hq), heads_of(g), :], wq_s.at[k + e], sem)
                for k in (0, 2)] + [pltpu.make_async_copy(sk_hbm.at[chans_of(2 * g + e), :], sk_s.at[e], sem)]

    def start(copies):
        for cp in copies:
            cp.start()

    def wait(copies):
        for cp in copies:
            cp.wait()

    wrows = T * HG // 2

    def stage(k, w):
        u = pltpu.bitcast(w.reshape(T * HG, DH), U32)
        w32[k * wrows:(k + 1) * wrows, :] = u
        return [u[b:b + T // 2] for b in range(0, wrows, T // 2)]

    def rhs_operands(k1, k2, p, put):
        blocks = [v for k in (k1, k2) for v in _halves(w32[pl.ds(k * wrows + p, T, stride=HG // 2), :])]
        ops = [_operand(spec, lambda b: blocks[b]) for spec in _RHS]
        for n in range(7):
            put(n, ops[n].astype(BF))
        return [_cat(ops[n][b:b + 16] for n in (0, 2, 5, 6)) for b in range(0, T, 16)]

    def wkv_operands(p):
        deps = []
        for t in range(2):
            def put(n, v):
                wkv7[p, 2 * n + t] = v
            deps += rhs_operands(t, 2 + t, p, put)
        return deps

    def lhs_operands(tile, dst, nk, which):
        step = 32

        def body(i, _):
            for r in range(0, T, step):
                rows = [pl.ds(pl.multiple_of(i * 2 * T + h * T + r, step), step) for h in range(2)]
                out_rows = pl.ds(pl.multiple_of(i * T + r, step), step)
                for t in range(nk):
                    blocks = [tile(t + k * nk, rows[h]).astype(F32) for h in range(2) for k in range(2)]
                    for slot, n in enumerate(which):
                        dst[slot * nk + t, out_rows, :] = _operand(_LHS[n], lambda b: blocks[b]).astype(BF)
        lax.fori_loop(0, NB, body, None)

    start([cp_c(), cp_wkv(0, 0)] + cp_small() + cp_early(0, 0) + cp_late(0, 0) + [cp_wkv(0, 1)])
    k32[0:8, :] = jnp.zeros((8, T), U32)
    cp_c().wait()
    lhs_operands(lambda t, rows: c_s[rows, t * T:(t + 1) * T], c7, DC // 2 // T, range(7))
    cp_wkv(0, 0).wait()
    for k in range(4):
        stage(k, wkv_s[0, k * T:(k + 1) * T])
    wkv_operands(0)
    wait(cp_small())
    d_s[...] = d_in[...].astype(F32)
    taps = sh_in[...].astype(F32)
    for cb in range(NCB):
        sh_s[cb] = taps[:, cb * T:(cb + 1) * T]
    wait(cp_early(0, 0))
    start(cp_early(0, 1) + cp_late(0, 1) + [cp_wkv(1, 0)] + cp_x())

    def proj_iter(g, e):
        cb = 2 * g + e
        zero, after = _pacing(cb)
        cw = C // 2
        im0 = T + 8
        u0, k0 = 0, 4 * NCH

        pl.when(cb > 0)(lambda: wait(cp_early(g, e)))

        def phases(ref, j, w0, w1):
            return [v for w in range(w0, w1) for v in _halves(ref[pl.ds(8 + j * cw + w, PH, stride=4), :])]

        def spectrum(ph, slot):
            parts = []
            for r in range(4):
                v = _dot(fwd_s[r], _cat([ph[r], ph[r + 4]]).astype(BF)).reshape(16, 2, 8, T)
                parts.append((v[:, 0], v[:, 1]))
            for s, (re, im) in enumerate(_dft4(parts, -1)):
                uk_s[zero + slot + s, 0:T] = re.reshape(T, T)
                uk_s[zero + slot + s, im0:im0 + T] = im.reshape(T, T)

        def short_conv(j):
            k32[8 + j * cw:8 + (j + 1) * cw, :] = pltpu.bitcast(bk_s[e, j * C:(j + 1) * C, :], U32)
            v32[8 + j * cw:8 + (j + 1) * cw, :] = pltpu.bitcast(bv_s[e, j * C:(j + 1) * C, :], U32)
            kp = phases(k32, j, -2, 4)
            vp = phases(v32, j, 0, 4)
            w = sh_s[cb]
            kv = [_sum([kp[4 + r - t] * w[t:t + 1, :] for t in range(KS)]) * vp[r] for r in range(8)]
            for r in range(8):
                p_s[zero + 8 * j + r] = kv[r]
            return [_cat(v[b:b + 8] for v in kv) for b in range(0, PH, 8)]

        def spectrum_kv(j):
            spectrum([p_s[8 * j + r] for r in range(8)], u0 + 4 * j)

        def spectrum_kernel(j):
            for m in range(4 * j, 4 * j + 4):
                h32[8 + m * (T // 2):8 + (m + 1) * (T // 2), :] = (
                    pltpu.bitcast(sk_s[e, :, m * T:(m + 1) * T].T, U32))
            spectrum(phases(h32, j, 0, 4), k0 + 4 * j)

        product = {}

        def chunk_conv(i, k):
            def load(n):
                return uk_s[n, 8 * k:8 * k + 8], uk_s[n, im0 + 8 * k:im0 + 8 * k + 8]
            z = []
            for s in range(4):
                acc = None
                for j in range(i + 1):
                    ur, ui = load(u0 + 4 * j + s)
                    kr, ki = load(k0 + 4 * (i - j) + s)
                    if acc is None:
                        acc = (ur * kr - ui * ki, ur * ki + ui * kr)
                    else:
                        acc = (acc[0] + ur * kr - ui * ki, acc[1] + ur * ki + ui * kr)
                product[i, k, s] = acc
                if i > 0:
                    pr, pi = product[i - 1, k, s]
                    acc = (acc[0] - pi, acc[1] + pr) if k < 8 else (acc[0] + pi, acc[1] - pr)
                z.append(acc)
            return _dft4(z, 1)

        mirror = {}

        def conv_mirror(i, k):
            mirror[i, k] = chunk_conv(i, k + 8)

        def conv_fold(i, k):
            for r, w in enumerate(_fold(chunk_conv(i, k), mirror[i, k])):
                z_s[zero + 8 * i + r, 16 * k:16 * k + 16] = _cat(w).astype(BF)

        def inverse(i):
            skip = d_s[pl.ds(cb, 1), :]
            ys = []
            for r in range(8):
                y = _dot(inv_s[r], z_s[8 * i + r]) + p_s[8 * i + r] * skip
                ys.append(pltpu.bitcast(y.astype(BF).astype(F32), U32))
            for w in range(4):
                y32[cb, pl.ds(i * cw + w, PH, stride=4), :] = (ys[2 * w] >> 16) | (ys[2 * w + 1] & HI16)

        def stage_wq():
            return [d for r in range(2) for h in range(2)
                    for d in stage(4 + 2 * r + h, wq_s[2 * h + e, r * T:(r + 1) * T])]

        def wq_operands():
            deps = []
            for r in range(2):
                for p in range(HG // 2):
                    def put(n, v):
                        wq7[(p * 7 + n) * 4 + 2 * e + r] = v
                    deps += rhs_operands(4 + 2 * r, 5 + 2 * r, p, put)
            return deps

        def stage_next_wkv():
            return [d for k in range(4) for d in stage(k, wkv_s[1 - e, k * T:(k + 1) * T])]

        def project(step, deps, tasks):
            p, i = divmod(step, NB)

            def prod(n):
                pos = _ORDER.index(n)
                terms = []
                for t in range(2):
                    lhs = c7[2 * n + t, i * T:(i + 1) * T, :]
                    for k, dep in enumerate(deps):
                        if k * 14 // len(deps) == 2 * pos + t:
                            lhs = after(lhs, dep)
                    terms.append(_dot(lhs, wkv7[p, 2 * n + t]))
                r = _sum(terms)
                for k, task in enumerate(tasks):
                    if k * 7 // len(tasks) == pos:
                        uk_s[zero, im0 + T:im0 + T + 8] = r[0:8]
                        task()
                if step == NB and pos == 3:
                    wait(cp_late(g, e))
                    pltpu.make_async_copy(wkv_s.at[1 - e], wkv_s.at[1 - e], sems.at[6 - e]).wait()
                return r

            for k, v in enumerate(_strassen(prod)):
                tile = 2 * i + k // 2
                kv_s[e * HG + 2 * p + k % 2, tile * T:(tile + 1) * T, :] = v.astype(BF)

        nsteps = HG // 2 * NB
        u_at, k_at = (2, 4, 6, 8), (10, 10, 12, 12)
        jobs = [(1, 7, lambda: wkv_operands(1)), (9, 15, lambda: wkv_operands(2) + wkv_operands(3)),
                (9, 14, stage_wq), (14, nsteps, wq_operands),
                (17, 24, stage_next_wkv), (24, nsteps, lambda: wkv_operands(0))]
        convs = [(first, last, lambda j=j: short_conv(j))
                 for j, (first, last) in enumerate(zip((0,) + u_at, u_at))]
        tasks = [lambda f=f, i=i, k=k: f(i, k)
                 for k in range(8) for i in range(NCH) for f in (conv_mirror, conv_fold)]

        def due(step, spec, live):
            live += [(last, job()) for first, last, job in spec if first == step]
            out = []
            for last, deps in live:
                n = -(-len(deps) // max(last - step, 1))
                out = _weave(out, deps[:n])
                del deps[:n]
            return out

        live_convs, live_jobs = [], []
        for step in range(nsteps):
            n = -(-len(tasks) // max(nsteps - 4 - step, 1)) if step >= k_at[-1] else 0
            project(step, _weave(due(step, convs, live_convs), due(step, jobs, live_jobs)), tasks[:n])
            del tasks[:n]
            for j in range(NCH):
                if u_at[j] == step + 1:
                    spectrum_kv(j)
                if k_at[j] == step + 1:
                    spectrum_kernel(j)
        for i in range(NCH):
            inverse(i)

    def head_pair(g, p):
        pair = g * (HG // 2) + p
        zero, after = _pacing(pair)
        scale = np.float32(DH ** -0.5 * np.log2(np.e))
        causal = lax.broadcasted_iota(jnp.int32, (T, T), 1) <= lax.broadcasted_iota(jnp.int32, (T, T), 0)
        nk = M // 2 // T
        row_max, inv_sum, ctx, stored = {}, {}, {}, {}
        tiles = [0]
        order = (7, 0, 5, 1, 6, 4, 3, 2)
        q_at, lag = (1, 5), 5

        def q_buf(i):
            return (q0, q1, q2, q3)[order.index(i) % 4]

        def s_buf(n):
            return (s0, s1, s2)[n % 3]

        def project_q(i, deps=None):
            def lhs(n, t):
                if n in _SUMS:
                    return x5[_SUMS.index(n) * nk + t, i * T:(i + 1) * T, :]
                h = n - 2
                v = x_s[t + h * nk, (2 * i + h) * T:(2 * i + h + 1) * T, :]
                if deps is not None and t == 0:
                    v = after(v, deps[(1 - h) * T // 2:(2 - h) * T // 2])
                return v
            blocks = _strassen(lambda n: _sum([_dot(lhs(n, t), wq7[(p * 7 + n) * nk + t]) for t in range(nk)]))
            tiles[0] += 7 * nk
            for k, v in enumerate(blocks):
                q_buf(i)[zero + k] = (v * scale).astype(BF)

        def scores(n, t, e):
            m = None
            for j in range(t + 1):
                s = _dot_nt(q_buf(t // 2)[2 * (t % 2) + e], kv_s[2 * p + e, j * T:(j + 1) * T, :])
                tiles[0] += 1
                if j == t:
                    s = jnp.where(causal, s, -1e30)
                s_buf(n)[zero + j] = s
                m = s if m is None else jnp.maximum(m, s)
            row_max[n] = jnp.broadcast_to(jnp.max(m, axis=1, keepdims=True), (T, T))

        def attend(n, t, e):
            m = row_max[n]
            if n >= lag:
                m = after(m, jnp.broadcast_to(inv_sum[n - lag], (T, T)))
            acc = l = None
            for j in range(t + 1):
                ex = jnp.exp2(s_buf(n)[j] - m)
                l = ex if l is None else l + ex
                if j > 0 and (tiles[0] % 4 == 3 or j == t):
                    ex = after(ex, l)
                r = _dot(ex.astype(BF), kv_s[HG + 2 * p + e, j * T:(j + 1) * T, :])
                tiles[0] += 1
                acc = r if acc is None else acc + r
            inv_sum[n] = pltpu.reciprocal(jnp.sum(l, axis=1, keepdims=True), full_range=False)
            i = t // 2
            ctx[i, 2 * (t % 2) + e] = acc * inv_sum[n]
            for k, spec in enumerate(_LHS):
                if (i, k) not in stored and all((i, b) in ctx for b in spec[::2]):
                    stored[i, k] = True
                    ctx7[pair * 7 + k, i * T:(i + 1) * T, :] = _operand(spec, lambda b: ctx[i, b]).astype(BF)

        rows = pl.ds(pl.multiple_of(pair * T, T), T)
        gw = gw_s[...].astype(F32)
        logit = _sum([x_s[t, rows, :].astype(F32) * gw[t:t + 1, :] for t in range(NCB)])
        gate = jnp.broadcast_to(jax.nn.sigmoid(jnp.sum(logit, axis=1, keepdims=True)), (T, T))
        g_s[rows, :] = gate

        units = [u for b in range(0, NB, 2) for e in range(2) for a in range(2)
                 for u in ((2 * order[b] + a, e), (2 * order[b + 1] + 1 - a, e))]
        project_q(order[0], logit)
        project_q(order[1], gate)
        scores(0, *units[0])
        scores(1, *units[1])
        for n, unit in enumerate(units):
            if n % 8 in q_at and n < len(units) - 8:
                project_q(order[n // 8 * 2 + 2 + q_at.index(n % 8)])
            if n + 2 < len(units):
                scores(n + 2, *units[n + 2])
            attend(n, *unit)

    def group(g, _):
        lax.fori_loop(0, 2, lambda e, _: proj_iter(g, e), None)

        @pl.when(g == 0)
        def _():
            wait(cp_x())
            lhs_operands(lambda t, rows: x_s[t, rows, :], x5, M // 2 // T, _SUMS)

        @pl.when(g < NG - 1)
        def _():
            start(cp_early(g + 1, 0) + cp_late(g + 1, 0) + [cp_wkv(g + 1, 1)]
                  + cp_early(g + 1, 1) + cp_late(g + 1, 1) + [cp_wkv((g + 2) & (NG - 1), 0)])

        start([cp_wo(2 * g), cp_wo(2 * g + 1)])
        lax.fori_loop(0, HG // 2, lambda p, _: head_pair(g, p), None)

    lax.fori_loop(0, NG, group, None)
    wait([cp_wo(cb) for cb in range(NCB)])

    def out_iter(k, _):
        rb = k & 1
        first = lax.shift_right_logical(k, 1) * 2
        cbs = (first, first + 1)

        def prod(n):
            terms = None
            for pair in range(H // 2):
                def block(b):
                    head = 2 * pair + b // 2
                    return wo_s[cbs[b % 2], head * DH:(head + 1) * DH, :]
                r = _dot(ctx7[pair * 7 + n, pl.ds(pl.multiple_of(rb * RO, RO), RO), :],
                         _operand(_RHS[n], block).astype(BF))
                terms = r if terms is None else terms + r
            return terms

        blocks = _strassen(prod)
        for b in (2, 0, 1, 3):
            cb = cbs[b % 2]
            for a in range(RO // T):
                tile = 2 * a + b // 2
                rows = pl.ds(pl.multiple_of(rb * 2 * RO + tile * T, T), T)
                words = pl.ds(pl.multiple_of(rb * RO + tile * (T // 2), T // 2), T // 2)
                gate = g_s[rows, :]
                conv = x_s[cb, rows, :].astype(F32) * pltpu.bitcast(y32[cb, words, :], BF).astype(F32)
                o_s[cb, rows, :] = (gate * blocks[b][a * T:(a + 1) * T] + (1.0 - gate) * conv).astype(BF)
        start([cp_out(cb, rb) for cb in cbs])

    lax.fori_loop(0, NCB, out_iter, None)
    wait([cp_out(cb, rb) for cb in range(NCB) for rb in range(2)])


@jax.jit
def pallas_gated_mix__compressed_kv_cla__ssm_conv_h3__prompt_kernel(
    A_x: jax.Array,
    A_c_kv: jax.Array,
    A_w_q: jax.Array,
    A_w_uk: jax.Array,
    A_w_uv: jax.Array,
    A_w_o: jax.Array,
    B_q: jax.Array,
    B_k: jax.Array,
    B_v: jax.Array,
    B_shift_k: jax.Array,
    B_ssm_k: jax.Array,
    B_ssm_D: jax.Array,
    gate_w: jax.Array,
):
    del B_q
    hbm = pl.BlockSpec(memory_space=pl.ANY)
    vmem = pltpu.VMEM
    pad = 64
    out = pl.pallas_call(
        _kernel,
        in_specs=[hbm] * 14,
        out_specs=hbm,
        out_shape=jax.ShapeDtypeStruct((S, M), BF),
        scratch_shapes=[
            vmem(_FWD.shape, BF), vmem(_INV.shape, BF),
            vmem((NCB, S, T), BF), vmem((S, DC), BF),
            vmem((4, M // 4, HG, DH), BF), vmem((2, DC, HG, DH), BF),
            vmem((NCB, H * DH, T), BF),
            vmem((2, S, T), BF), vmem((2, S, T), BF), vmem((2, T, S), BF),
            vmem((NCB, S, T), BF), vmem((NCB, S // 2 + pad, T), U32),
            vmem((2 * HG, S, DH), BF), vmem((7 * H // 2, S // 2, DH), BF),
            vmem((7 * HG // 2 * NCB // 2, T, DH), BF),
            vmem((5 * NCB // 2, S // 2, T), BF),
            vmem((7 * DC // T // 2, S // 2, T), BF),
            vmem((HG // 2, 14, T, DH), BF),
            vmem((8 * T * HG // 2 + pad, DH), U32),
            vmem((S, T), F32),
            *[vmem((S // 2 + pad, T), U32) for _ in range(3)],
            vmem((8 * NCH, T, T), BF),
            vmem((8 * NCH, 2 * T + 16, T), F32),
            vmem((8 * NCH, PH, T), F32),
            *[vmem((4, T, DH), BF) for _ in range(4)],
            *[vmem((NT, T, T), F32) for _ in range(3)],
            vmem((NCB, KS, T), F32), vmem((KS, M), BF),
            vmem((NCB, T), F32), vmem((NCB, T), BF), vmem((NCB, T), BF),
            pltpu.SemaphoreType.DMA((11,)),
        ],
        compiler_params=pltpu.CompilerParams(vmem_limit_bytes=120 * 2 ** 20),
    )(A_x.reshape(S, M), A_c_kv.reshape(S, DC), A_w_q, A_w_uk, A_w_uv, A_w_o.reshape(H * DH, M),
      B_k.reshape(S, M), B_v.reshape(S, M), B_ssm_k, B_shift_k.T,
      B_ssm_D.reshape(NCB, T), gate_w.reshape(NCB, T), _FWD, _INV)
    return out.reshape(1, S, M)
```
